```python
import jax
import jax.numpy as jnp

def _softmax(x, axis=-1):
    return jax.nn.softmax(x, axis=axis)
def _gelu(x):
    return jax.nn.gelu(x, approximate=True)
def _silu(x):
    return jax.nn.silu(x)
def _sigmoid(x):
    return jax.nn.sigmoid(x)
def _layernorm(x, axis=-1, eps=1e-5):
    m = jnp.mean(x, axis=axis, keepdims=True)
    v = jnp.var(x, axis=axis, keepdims=True)
    return (x - m) / jnp.sqrt(v + eps)
def _scatter_add(tgt, idx, src, axis=0):
    return tgt.at[idx].add(src)
def _segment_sum(src, seg, n):
    return jax.ops.segment_sum(src, seg, n)
class _Rng:
    def __init__(self, key):
        self._k = key
    def _next(self):
        self._k, sub = jax.random.split(self._k)
        return sub
    def normal(self, shape):
        return jax.random.normal(self._next(), shape, dtype=jnp.bfloat16)
    def randint(self, lo, hi, shape):
        return jax.random.randint(self._next(), shape, lo, hi, dtype=jnp.int32)
    def uniform(self, shape, lo=0.0, hi=1.0):
        return jax.random.uniform(self._next(), shape, jnp.bfloat16, lo, hi)
    def permutation(self, n):
        return jax.random.permutation(self._next(), n)


kernel_name = 'sequential_preLN__sliding_block__glu_gated_glu__prompt'

def _fwd_setup_inputs():
    _rng = _Rng(jax.random.key(int.from_bytes(__import__("os").urandom(4), "little")))
    _w = (lambda a: (lambda t: t.astype(jnp.bfloat16) if jnp.issubdtype(t.dtype, jnp.floating) else t)(jnp.asarray(a)))
    def _A_setup():
        B, S, D = 1, 2048, 512
        return {
            "x": _w((lambda *s: _rng.normal(s) * 0.05)(B, S, D)),
            "wqkv": _w((lambda *s: _rng.normal(s) * 0.05)(D, 3 * D)),
            "wo": _w((lambda *s: _rng.normal(s) * 0.05)(D, D)),
        }
    _A_in = _A_setup()

    def _B_setup():
        B, S, D, F = 1, 2048, 512, 1376
        return {
            "x": _w((lambda *s: _rng.normal(s) * 0.05)(B, S, D)),
            "w_gate": _w((lambda *s: _rng.normal(s) * 0.05)(D, F)),
            "w_up": _w((lambda *s: _rng.normal(s) * 0.05)(D, F)),
            "w_down": _w((lambda *s: _rng.normal(s) * 0.05)(F, D)),
        }
    _B_in = _B_setup()

    return {
        "A_x": _A_in["x"],
        "A_wqkv": _A_in["wqkv"],
        "A_wo": _A_in["wo"],
        "B_x": _B_in["x"],
        "B_w_gate": _B_in["w_gate"],
        "B_w_up": _B_in["w_up"],
        "B_w_down": _B_in["w_down"],
    }

def _fwd_reference(A_x, A_wqkv, A_wo, B_x, B_w_gate, B_w_up, B_w_down):
    def _A_ref(x, wqkv, wo):
        B, S, D = x.shape
        H = 32; Dh = D // H; W = 256
        qkv = (lambda x, *d: x.transpose(*d))((x @ wqkv).reshape(B, S, 3, H, Dh), 2, 0, 3, 1, 4)
        q, k, v = qkv[0], qkv[1], qkv[2]
        scores = jnp.einsum("bhqd,bhkd->bhqk", q, k) * (Dh ** -0.5)
        idx = jnp.arange(S)
        mask = (idx[:, None] - idx[None, :] >= 0) & (idx[:, None] - idx[None, :] < W)
        scores = jnp.where(mask[None, None], scores, -1e9)
        p = _softmax(scores, axis=-1)
        o = jnp.einsum("bhqk,bhkd->bhqd", p, v)
        return (lambda x, *d: x.transpose(*d))(o, 0, 2, 1, 3).reshape(B, S, D) @ wo

    def _B_ref(x, w_gate, w_up, w_down):
        g = jnp.einsum("bsd,df->bsf", x, w_gate)
        u = jnp.einsum("bsd,df->bsf", x, w_up)
        h = _sigmoid(g) * u
        return jnp.einsum("bsf,fd->bsd", h, w_down)

    x = A_x
    h = x + _A_ref(_layernorm(x, axis=-1), A_wqkv, A_wo)
    h2 = h + _B_ref(_layernorm(h, axis=-1), B_w_gate, B_w_up, B_w_down)
    return h2


def setup_inputs():
    _inp = _fwd_setup_inputs()
    _gk = jax.random.fold_in(jax.random.key(int.from_bytes(__import__("os").urandom(4), "little")), 2**31 - 1)
    _shapes = [[1, 2048, 512]]
    _dtypes = ['bfloat16']
    _gks = jax.random.split(_gk, len(_shapes))
    _gs = [jax.random.normal(k, s, dtype=jnp.dtype(d)) * 0.05 for k, s, d in zip(_gks, _shapes, _dtypes)]
    _inp["grad_out"] = _gs[0]
    return _inp

def reference(A_x, A_wqkv, A_wo, B_w_gate, B_w_up, B_w_down, B_x, grad_out):
    _const = dict(B_x=B_x)
    def _f(*_d):
        return _fwd_reference(**{'A_x': _d[0], 'A_wqkv': _d[1], 'A_wo': _d[2], 'B_w_gate': _d[3], 'B_w_up': _d[4], 'B_w_down': _d[5], **_const})
    _out, _vjp = jax.vjp(_f, A_x, A_wqkv, A_wo, B_w_gate, B_w_up, B_w_down)
    _grads = _vjp(grad_out)
    _out0 = jnp.asarray(_out)
    return (_out0, *[jnp.asarray(_g) for _g in _grads])
```

```python
import functools

import jax
import jax.numpy as jnp
from jax import lax
import jax.experimental.pallas as pl
import jax.experimental.pallas.tpu as pltpu

_H = 32
_DH = 16
_W = 256
_EPS = 1e-5
_NEG = -1e9

_T = 256
_QB = 64

_F32 = jnp.float32
_BF16 = jnp.bfloat16

_NN = (((1,), (0,)), ((), ()))
_NT = (((1,), (1,)), ((), ()))
_TN = (((0,), (0,)), ((), ()))


def _dot(a, b, dims):
    return lax.dot_general(a, b, dims, preferred_element_type=_F32)


def _ln_stats(x):
    m = jnp.mean(x, axis=-1, keepdims=True)
    xc = x - m
    v = jnp.mean(xc * xc, axis=-1, keepdims=True)
    r = lax.rsqrt(v + _EPS)
    return xc * r, r


def _ln_bwd(dy, xhat, r):
    a = jnp.mean(dy, axis=-1, keepdims=True)
    b = jnp.mean(dy * xhat, axis=-1, keepdims=True)
    return r * (dy - a - xhat * b)


def _kernel(x_ref, xl_ref, dy_ref, wqkv_ref, wo_ref, wg_ref, wu_ref, wd_ref,
            out_ref, dx_ref, dwqkv_ref, dwo_ref, dwg_ref, dwu_ref, dwd_ref,
            q_s, k_s, v_s, kt_s, vt_s, p_s, ot_s, do_s, dqt_s, dq_s, dk_s, dv_s,
            dh_s, aqkv, ao, ag, au, ad,
            *, S, D, T, QB):
    nblk = S // T
    HP = 128 // QB
    NG = D // 128
    NP = 8 // HP
    R = _W + QB
    scale = _DH ** -0.5
    s = pl.program_id(0)

    @pl.when(s == 0)
    def _init():
        k_s[:, pl.ds(0, _W), :] = jnp.zeros((NG, _W, 128), _BF16)
        v_s[:, pl.ds(0, _W), :] = jnp.zeros((NG, _W, 128), _BF16)
        kt_s[:, pl.ds(0, _W)] = jnp.zeros((D, _W), _BF16)
        vt_s[:, pl.ds(0, _W)] = jnp.zeros((D, _W), _BF16)
        dk_s[...] = jnp.zeros(dk_s.shape, _F32)
        dv_s[...] = jnp.zeros(dv_s.shape, _F32)
        aqkv[...] = jnp.zeros(aqkv.shape, _F32)
        ao[...] = jnp.zeros(ao.shape, _F32)
        ag[...] = jnp.zeros(ag.shape, _F32)
        au[...] = jnp.zeros(au.shape, _F32)
        ad[...] = jnp.zeros(ad.shape, _F32)

    row128 = lax.broadcasted_iota(jnp.int32, (128, 128), 0)
    lane128 = lax.broadcasted_iota(jnp.int32, (128, 128), 1)
    rq = lax.broadcasted_iota(jnp.int32, (QB, 128), 0)
    lq = lax.broadcasted_iota(jnp.int32, (QB, 128), 1) % QB
    old_valid = rq > lq
    rw = lax.broadcasted_iota(jnp.int32, (_W, 128), 0)
    lw = lax.broadcasted_iota(jnp.int32, (_W, 128), 1) % QB

    def head_mask(pr):
        return (row128 // QB + pr * HP) == (lane128 // _DH)

    def stacked(src_ref, grp, pr, qrow):
        sub = src_ref[grp, pl.ds(qrow, QB), :]
        st = jnp.concatenate([sub] * HP, axis=0)
        return jnp.where(head_mask(pr), st, 0.0).astype(_BF16)

    def combine(full):
        edge = jnp.where(old_valid, full[0:QB], full[_W:_W + QB])
        return jnp.concatenate([edge, full[QB:_W]], axis=0)

    def expand(c):
        e = c[0:QB]
        lo = jnp.where(old_valid, e, 0.0)
        hi = jnp.where(old_valid, 0.0, e)
        return jnp.concatenate([lo, c[QB:_W], hi], axis=0).astype(_BF16)

    def place_t(dst_ref, tile, grp, pr, g128, sb):
        for hh in range(HP):
            piece = tile[hh * _DH:(hh + 1) * _DH, hh * QB:(hh + 1) * QB]
            r0 = pl.multiple_of(grp * 128 + (pr * HP + hh) * _DH, _DH)
            c0 = g128 * 128 + sb * QB
            dst_ref[pl.ds(r0, _DH), c0:c0 + QB] = piece

    @pl.when(s < nblk)
    def _main():
        row0 = pl.multiple_of(s * T, T)
        prow0 = pl.multiple_of(s * T + _W, 128)
        x = x_ref[...].astype(_F32)
        ln1, _ = _ln_stats(x)
        qkv = _dot(ln1.astype(_BF16), wqkv_ref[...], _NN)
        for g in range(NG):
            q_s[g] = qkv[:, g * 128:(g + 1) * 128] * scale
            k_s[g, pl.ds(prow0, T), :] = qkv[:, D + g * 128:D + (g + 1) * 128].astype(_BF16)
            v_s[g, pl.ds(prow0, T), :] = qkv[:, 2 * D + g * 128:2 * D + (g + 1) * 128].astype(_BF16)
        kt_s[:, pl.ds(prow0, T)] = qkv[:, D:2 * D].T.astype(_BF16)
        vt_s[:, pl.ds(prow0, T)] = qkv[:, 2 * D:3 * D].T.astype(_BF16)

        for g128 in range(T // 128):
            base = pl.multiple_of(row0 + g128 * 128, 128)
            for sb in range(HP):
                i0 = base + sb * QB
                qrow = g128 * 128 + sb * QB
                kvalid = jnp.logical_or(rw + (i0 - _W) >= 0,
                                        jnp.logical_and(rw < QB, rw <= lw))

                def fwd_tile(idx, carry, g128=g128, sb=sb, i0=i0, qrow=qrow, kvalid=kvalid, base=base):
                    grp = idx // NP
                    pr = idx % NP
                    qb = stacked(q_s, grp, pr, qrow)
                    kwin = k_s[grp, pl.ds(pl.multiple_of(i0, QB), R), :]
                    st = _dot(kwin, qb, _NT)
                    c = combine(st)
                    c = jnp.where(kvalid, c, _NEG)
                    m = jnp.max(c, axis=0, keepdims=True)
                    e = jnp.exp(c - m)
                    l = jnp.sum(e, axis=0, keepdims=True)
                    p = e * (1.0 / l)
                    pf = expand(p)
                    tid = (g128 * HP + sb) * (NG * NP) + idx
                    p_s[tid] = pf
                    r0 = pl.multiple_of(grp * 128 + pr * HP * _DH, HP * _DH)
                    vt = vt_s[pl.ds(r0, HP * _DH), pl.ds(base, 128 + _W)]
                    vt = vt[:, sb * QB:sb * QB + R]
                    ot = _dot(vt, pf, _NN)
                    place_t(ot_s, ot, grp, pr, g128, sb)
                    return carry

                lax.fori_loop(0, NG * NP, fwd_tile, 0)

        ot = ot_s[...]
        otb = ot.astype(_BF16)
        o = ot.T.astype(_BF16)
        h = x + _dot(o, wo_ref[...], _NN)
        ln2, r2 = _ln_stats(h)
        ln2b = ln2.astype(_BF16)
        g_ = _dot(ln2b, wg_ref[...], _NN)
        u_ = _dot(ln2b, wu_ref[...], _NN)
        sg = jax.nn.sigmoid(g_)
        hh_b = (sg * u_).astype(_BF16)
        out_ref[...] = (h + _dot(hh_b, wd_ref[...], _NN)).astype(out_ref.dtype)

        dyb = dy_ref[...]
        dy = dyb.astype(_F32)
        ad[...] += _dot(hh_b, dyb, _TN)
        dhh = _dot(dyb, wd_ref[...], _NT)
        dgb = (dhh * u_ * sg * (1.0 - sg)).astype(_BF16)
        dub = (dhh * sg).astype(_BF16)
        ag[...] += _dot(ln2b, dgb, _TN)
        au[...] += _dot(ln2b, dub, _TN)
        dln2 = _dot(dgb, wg_ref[...], _NT) + _dot(dub, wu_ref[...], _NT)
        dh = dy + _ln_bwd(dln2, ln2, r2)
        dh_s[pl.ds(row0, T), :] = dh
        dhb = dh.astype(_BF16)
        ao[...] += _dot(otb, dhb, _NN)
        do = _dot(dhb, wo_ref[...], _NT)
        for g in range(NG):
            do_s[g] = do[:, g * 128:(g + 1) * 128]

        for g128 in range(T // 128):
            base = pl.multiple_of(row0 + g128 * 128, 128)
            for sb in range(HP):
                i0 = base + sb * QB
                qrow = g128 * 128 + sb * QB

                def bwd_tile(idx, carry, g128=g128, sb=sb, i0=i0, qrow=qrow, base=base):
                    grp = idx // NP
                    pr = idx % NP
                    win = pl.ds(pl.multiple_of(i0, QB), R)
                    tid = (g128 * HP + sb) * (NG * NP) + idx
                    pf = p_s[tid]
                    dob = stacked(do_s, grp, pr, qrow)
                    qb = stacked(q_s, grp, pr, qrow)
                    vwin = v_s[grp, win, :]
                    dpt = _dot(vwin, dob, _NT)
                    dpc = combine(dpt)
                    pc = combine(pf.astype(_F32))
                    delta = jnp.sum(pc * dpc, axis=0, keepdims=True)
                    dsc = pc * (dpc - delta)
                    dsf = expand(dsc)
                    dv_s[grp, win, :] += _dot(pf, dob, _NN)
                    dk_s[grp, win, :] += _dot(dsf, qb, _NN)
                    r0 = pl.multiple_of(grp * 128 + pr * HP * _DH, HP * _DH)
                    kt = kt_s[pl.ds(r0, HP * _DH), pl.ds(base, 128 + _W)]
                    kt = kt[:, sb * QB:sb * QB + R]
                    dqt = _dot(kt, dsf, _NN) * scale
                    place_t(dqt_s, dqt, grp, pr, g128, sb)
                    return carry

                lax.fori_loop(0, NG * NP, bwd_tile, 0)

        dq_s[pl.ds(row0, T), :] = dqt_s[...].T.astype(_BF16)

    @pl.when(s > 0)
    def _lag():
        lrow0 = pl.multiple_of((s - 1) * T, T)
        lprow0 = pl.multiple_of((s - 1) * T + _W, 128)
        xl = xl_ref[...].astype(_F32)
        ln1, r1 = _ln_stats(xl)
        ln1b = ln1.astype(_BF16)
        parts = [dq_s[pl.ds(lrow0, T), :]]
        for g in range(NG):
            parts.append(dk_s[g, pl.ds(lprow0, T), :].astype(_BF16))
        for g in range(NG):
            parts.append(dv_s[g, pl.ds(lprow0, T), :].astype(_BF16))
        dqkv = jnp.concatenate(parts, axis=1)
        aqkv[...] += _dot(ln1b, dqkv, _TN)
        dln1 = _dot(dqkv, wqkv_ref[...], _NT)
        dx = dh_s[pl.ds(lrow0, T), :] + _ln_bwd(dln1, ln1, r1)
        dx_ref[...] = dx.astype(dx_ref.dtype)

    @pl.when(s == nblk)
    def _fin():
        dwqkv_ref[...] = aqkv[...].astype(dwqkv_ref.dtype)
        dwo_ref[...] = ao[...].astype(dwo_ref.dtype)
        dwg_ref[...] = ag[...].astype(dwg_ref.dtype)
        dwu_ref[...] = au[...].astype(dwu_ref.dtype)
        dwd_ref[...] = ad[...].astype(dwd_ref.dtype)


@jax.jit
def pallas_sequential_preLN__sliding_block__glu_gated_glu__prompt_kernel(
    A_x: jax.Array,
    A_wqkv: jax.Array,
    A_wo: jax.Array,
    B_x: jax.Array,
    B_w_gate: jax.Array,
    B_w_up: jax.Array,
    B_w_down: jax.Array,
    grad_out: jax.Array,
):
    del B_x
    _, S, D = A_x.shape
    F = B_w_gate.shape[1]
    T, QB = _T, _QB
    nblk = S // T
    HP = 128 // QB
    NG = D // 128
    NP = 8 // HP
    R = _W + QB
    ntile = (T // QB) * NG * NP

    cur = lambda s: (0, jnp.minimum(s, nblk - 1), 0)
    lag = lambda s: (0, jnp.maximum(s - 1, 0), 0)
    whole = lambda s: (0, 0)

    in_specs = [
        pl.BlockSpec((None, T, D), cur),
        pl.BlockSpec((None, T, D), lag),
        pl.BlockSpec((None, T, D), cur),
        pl.BlockSpec((D, 3 * D), whole),
        pl.BlockSpec((D, D), whole),
        pl.BlockSpec((D, F), whole),
        pl.BlockSpec((D, F), whole),
        pl.BlockSpec((F, D), whole),
    ]
    out_specs = [
        pl.BlockSpec((None, T, D), cur),
        pl.BlockSpec((None, T, D), lag),
        pl.BlockSpec((D, 3 * D), whole),
        pl.BlockSpec((D, D), whole),
        pl.BlockSpec((D, F), whole),
        pl.BlockSpec((D, F), whole),
        pl.BlockSpec((F, D), whole),
    ]
    out_shape = [
        jax.ShapeDtypeStruct((1, S, D), A_x.dtype),
        jax.ShapeDtypeStruct((1, S, D), A_x.dtype),
        jax.ShapeDtypeStruct((D, 3 * D), A_wqkv.dtype),
        jax.ShapeDtypeStruct((D, D), A_wo.dtype),
        jax.ShapeDtypeStruct((D, F), B_w_gate.dtype),
        jax.ShapeDtypeStruct((D, F), B_w_up.dtype),
        jax.ShapeDtypeStruct((F, D), B_w_down.dtype),
    ]
    scratch_shapes = [
        pltpu.VMEM((NG, T, 128), _F32),
        pltpu.VMEM((NG, S + _W, 128), _BF16),
        pltpu.VMEM((NG, S + _W, 128), _BF16),
        pltpu.VMEM((D, S + _W), _BF16),
        pltpu.VMEM((D, S + _W), _BF16),
        pltpu.VMEM((ntile, R, 128), _BF16),
        pltpu.VMEM((D, T), _F32),
        pltpu.VMEM((NG, T, 128), _F32),
        pltpu.VMEM((D, T), _F32),
        pltpu.VMEM((S, D), _BF16),
        pltpu.VMEM((NG, S + _W, 128), _F32),
        pltpu.VMEM((NG, S + _W, 128), _F32),
        pltpu.VMEM((S, D), _F32),
        pltpu.VMEM((D, 3 * D), _F32),
        pltpu.VMEM((D, D), _F32),
        pltpu.VMEM((D, F), _F32),
        pltpu.VMEM((D, F), _F32),
        pltpu.VMEM((F, D), _F32),
    ]
    return pl.pallas_call(
        functools.partial(_kernel, S=S, D=D, T=T, QB=QB),
        grid=(nblk + 1,),
        in_specs=in_specs,
        out_specs=out_specs,
        out_shape=out_shape,
        scratch_shapes=scratch_shapes,
        compiler_params=pltpu.CompilerParams(
            dimension_semantics=("arbitrary",),
            vmem_limit_bytes=110 * 1024 * 1024,
        ),
    )(A_x, A_x, grad_out, A_wqkv, A_wo, B_w_gate, B_w_up, B_w_down)
```

```python
import functools

import jax
import jax.numpy as jnp
from jax import lax
import jax.experimental.pallas as pl
import jax.experimental.pallas.tpu as pltpu

_H = 32
_DH = 16
_W = 256
_EPS = 1e-5
_NEG = -1e9
_QB = 128
_R = _W + _QB

_T = 256
_HU = 8

_F32 = jnp.float32
_BF16 = jnp.bfloat16

_NN = (((1,), (0,)), ((), ()))
_NT = (((1,), (1,)), ((), ()))
_TN = (((0,), (0,)), ((), ()))


def _dot(a, b, dims):
    return lax.dot_general(a, b, dims, preferred_element_type=_F32)


def _pk(x):
    return pltpu.bitcast(x.astype(_BF16), jnp.uint32)


def _upk(x):
    return pltpu.bitcast(x, _BF16)


def _ln_stats(x):
    m = jnp.mean(x, axis=-1, keepdims=True)
    xc = x - m
    v = jnp.mean(xc * xc, axis=-1, keepdims=True)
    r = lax.rsqrt(v + _EPS)
    return xc * r, r


def _ln_bwd(dy, xhat, r):
    a = jnp.mean(dy, axis=-1, keepdims=True)
    b = jnp.mean(dy * xhat, axis=-1, keepdims=True)
    return r * (dy - a - xhat * b)


def _kernel(x_ref, xl_ref, dy_ref, wqkv_ref, wo_ref, wgt_ref, wut_ref, wd_ref,
            out_ref, dx_ref, dwqkv_ref, dwo_ref, dwgt_ref, dwut_ref, dwd_ref,
            wq_s, wdo_s, k_s, v_s, kt_s, vt_s, e_s, st_s, be_s, dl_s, ot_s,
            ds0_s, ds1_s, ds2_s, ds3_s, dqt_s,
            dkt_s, dvt_s, dh_s, aqkv, ao, ag, au, ad,
            *, S, D, T, HU):
    nblk = S // T
    QB, R = _QB, _R
    NG = D // 128
    UPQ = _H // HU
    NQB = T // QB
    NU = NQB * UPQ
    scale = _DH ** -0.5
    s = pl.program_id(0)
    ds_sl = (ds0_s, ds1_s, ds2_s, ds3_s)

    @pl.when(s == 0)
    def _init():
        wq_s[...] = jnp.zeros(wq_s.shape, jnp.uint32)
        wdo_s[...] = jnp.zeros(wdo_s.shape, jnp.uint32)
        k_s[:, pl.ds(0, _W // 2), :] = jnp.zeros((NG, _W // 2, 128), jnp.uint32)
        v_s[:, pl.ds(0, _W // 2), :] = jnp.zeros((NG, _W // 2, 128), jnp.uint32)
        kt_s[:, pl.ds(0, _W)] = jnp.zeros((D, _W), _BF16)
        vt_s[:, pl.ds(0, _W)] = jnp.zeros((D, _W), _BF16)
        dkt_s[...] = jnp.zeros(dkt_s.shape, _F32)
        dvt_s[...] = jnp.zeros(dvt_s.shape, _F32)
        aqkv[...] = jnp.zeros(aqkv.shape, _F32)
        ao[...] = jnp.zeros(ao.shape, _F32)
        ag[...] = jnp.zeros(ag.shape, _F32)
        au[...] = jnp.zeros(au.shape, _F32)
        ad[...] = jnp.zeros(ad.shape, _F32)

    def old_valid():
        rq = lax.broadcasted_iota(jnp.int32, (QB, QB), 0)
        lq = lax.broadcasted_iota(jnp.int32, (QB, QB), 1)
        return rq > lq

    def unit_coords(u, row0):
        qb = u // UPQ
        h0 = (u % UPQ) * HU
        grp = h0 // 8
        qcol = pl.multiple_of(qb * QB, QB)
        i0 = pl.multiple_of(row0 + qb * QB, QB)
        return qb, h0, grp, qcol, i0

    def interleave(*streams):
        n = max(len(st) for st in streams)
        for i in range(n):
            for st in streams:
                lo = (i * len(st)) // n
                hi = ((i + 1) * len(st)) // n
                for f in st[lo:hi]:
                    f()

    def chunk_scores(src_s, grp, i0, w, edge):
        hb = pl.multiple_of(i0 // 2, 64)
        if edge:
            lhs = jnp.concatenate([_upk(src_s[grp, pl.ds(hb, 64), :]),
                                   _upk(src_s[grp, pl.ds(hb + _W // 2, 64), :])], axis=0)
            full = _dot(lhs, w, _NN)
            return jnp.where(old_valid(), full[0:QB], full[QB:2 * QB])
        return _dot(_upk(src_s[grp, pl.ds(hb + 64, 64), :]), w, _NN)

    def store_expanded(dst, val, edge):
        if edge:
            ov = old_valid()
            dst[0:QB, :] = jnp.where(ov, val, 0.0).astype(_BF16)
            dst[_W:_W + QB, :] = jnp.where(ov, 0.0, val).astype(_BF16)
        else:
            dst[QB:_W, :] = val.astype(_BF16)

    @pl.when(s < nblk)
    def _main():
        row0 = pl.multiple_of(s * T, T)
        prow0 = pl.multiple_of(s * T + _W, 128)
        prow0h = pl.multiple_of((s * T + _W) // 2, 64)
        x = x_ref[...].astype(_F32)
        ln1, _ = _ln_stats(x)
        qkv = _dot(ln1.astype(_BF16), wqkv_ref[...], _NN)
        for g in range(NG):
            k_s[g, pl.ds(prow0h, T // 2), :] = _pk(qkv[:, D + g * 128:D + (g + 1) * 128])
            v_s[g, pl.ds(prow0h, T // 2), :] = _pk(qkv[:, 2 * D + g * 128:2 * D + (g + 1) * 128])
        qt = (qkv[:, 0:D].T * scale).astype(_BF16)
        for qb in range(NQB):
            for h in range(_H):
                hr = (h % 8) * _DH
                wq_s[qb * _H + h, hr // 2:(hr + _DH) // 2, :] = _pk(qt[h * _DH:(h + 1) * _DH, qb * QB:(qb + 1) * QB])
        kt_s[:, pl.ds(prow0, T)] = qkv[:, D:2 * D].T.astype(_BF16)
        vt_s[:, pl.ds(prow0, T)] = qkv[:, 2 * D:3 * D].T.astype(_BF16)

        def fa_steps(u, first):
            qb, h0, grp, qcol, i0 = unit_coords(u, row0)

            def mk(j, edge):
                def f():
                    w = _upk(wq_s[qb * _H + h0 + j])
                    c = chunk_scores(k_s, grp, i0, w, edge)
                    if first:
                        rw = lax.broadcasted_iota(jnp.int32, (QB, QB), 0) + (0 if edge else QB)
                        kvalid = rw + (i0 - _W) >= 0
                        if edge:
                            kvalid = jnp.logical_or(kvalid, jnp.logical_not(old_valid()))
                        c = jnp.where(kvalid, c, _NEG)
                    m = jnp.max(c, axis=0, keepdims=True)
                    e = jnp.exp(c - m)
                    l = jnp.sum(e, axis=0, keepdims=True)
                    store_expanded(e_s.at[u, j], e, edge)
                    t = 0 if edge else 1
                    st_s[u, j, 2 * t:2 * t + 1, :] = m
                    st_s[u, j, 2 * t + 1:2 * t + 2, :] = l
                return f

            return [mk(j, edge) for j in range(HU) for edge in (True, False)]

        def fc_steps(u):
            qb, h0, grp, qcol, i0 = unit_coords(u, row0)

            def mk(j):
                def f():
                    r0 = pl.multiple_of((h0 + j) * _DH, _DH)
                    stt = st_s[u, j]
                    me, le, mm, lm = stt[0:1], stt[1:2], stt[2:3], stt[3:4]
                    m = jnp.maximum(me, mm)
                    ae = jnp.exp(me - m)
                    am = jnp.exp(mm - m)
                    linv = 1.0 / (ae * le + am * lm)
                    be = ae * linv
                    bm = am * linv
                    be_s[u, j, 0:1, :] = be
                    be_s[u, j, 1:2, :] = bm
                    vt = vt_s[pl.ds(r0, _DH), pl.ds(i0, R)]
                    oe = (_dot(vt[:, 0:QB], e_s[u, j, 0:QB, :], _NN)
                          + _dot(vt[:, _W:R], e_s[u, j, _W:R, :], _NN))
                    om = _dot(vt[:, QB:_W], e_s[u, j, QB:_W, :], _NN)
                    ot_s[pl.ds(r0, _DH), pl.ds(qcol, QB)] = oe * be + om * bm
                return f

            return [mk(j) for j in range(HU)]

        def fwd_attn(first):
            def hb(u, head, tail):
                a = [] if tail else (fa_steps(u + 2, first) + fa_steps(u + 3, first))
                c = fc_steps(u) + fc_steps(u + 1)
                interleave(a, c)

            interleave(fa_steps(0, first) + fa_steps(1, first))

            def body(k, carry):
                hb(2 * k, False, False)
                return carry

            lax.fori_loop(0, NU // 2 - 1, body, 0)
            hb(NU - 2, False, True)

        @pl.when(row0 < _W)
        def _():
            fwd_attn(True)

        @pl.when(row0 >= _W)
        def _():
            fwd_attn(False)

        ot = ot_s[...]
        otb = ot.astype(_BF16)
        o = ot.T.astype(_BF16)
        h = x + _dot(o, wo_ref[...], _NN)
        ln2, r2 = _ln_stats(h)
        ln2b = ln2.astype(_BF16)
        g_ = _dot(ln2b, wgt_ref[...], _NT)
        u_ = _dot(ln2b, wut_ref[...], _NT)
        sg = jax.nn.sigmoid(g_)
        hh_b = (sg * u_).astype(_BF16)
        out_ref[...] = (h + _dot(hh_b, wd_ref[...], _NN)).astype(out_ref.dtype)

        dyb = dy_ref[...]
        dy = dyb.astype(_F32)
        ad[...] += _dot(hh_b, dyb, _TN)
        dhh = _dot(dyb, wd_ref[...], _NT)
        dgb = (dhh * u_ * sg * (1.0 - sg)).astype(_BF16)
        dub = (dhh * sg).astype(_BF16)
        ag[...] += _dot(ln2b, dgb, _TN)
        au[...] += _dot(ln2b, dub, _TN)
        dln2 = _dot(dgb, wgt_ref[...], _NN) + _dot(dub, wut_ref[...], _NN)
        dh = dy + _ln_bwd(dln2, ln2, r2)
        dh_s[pl.ds(row0, T), :] = dh
        dhb = dh.astype(_BF16)
        ao[...] += _dot(otb, dhb, _NN)
        dot = _dot(wo_ref[...], dhb, _NT)

        prod = ot * dot
        for u in range(NU):
            qb = u // UPQ
            h0 = (u % UPQ) * HU
            for j in range(HU):
                hd = h0 + j
                hr = (hd % 8) * _DH
                blk = dot[hd * _DH:(hd + 1) * _DH, qb * QB:(qb + 1) * QB]
                pb = prod[hd * _DH:(hd + 1) * _DH, qb * QB:(qb + 1) * QB]
                delta = jnp.sum(pb, axis=0, keepdims=True)
                for t in range(2):
                    bt = be_s[u, j, t:t + 1, :]
                    wdo_s[t, qb * _H + hd, hr // 2:(hr + _DH) // 2, :] = _pk(blk * bt)
                    dl_s[u, j, t:t + 1, :] = delta * bt

        def ba_steps(u, slot):
            qb, h0, grp, qcol, i0 = unit_coords(u, row0)

            def mk(j, edge):
                def f():
                    t = 0 if edge else 1
                    w = _upk(wdo_s[t, qb * _H + h0 + j])
                    dpc = chunk_scores(v_s, grp, i0, w, edge) - dl_s[u, j, t:t + 1, :]
                    if edge:
                        p = e_s[u, j, 0:QB, :].astype(_F32) + e_s[u, j, _W:R, :].astype(_F32)
                    else:
                        p = e_s[u, j, QB:_W, :].astype(_F32)
                    store_expanded(ds_sl[slot].at[j], p * dpc, edge)
                return f

            return [mk(j, edge) for j in range(HU) for edge in (True, False)]

        def bc_steps(u, slot):
            qb, h0, grp, qcol, i0 = unit_coords(u, row0)
            win = pl.ds(i0, R)

            def mk(j):
                def f():
                    r0 = pl.multiple_of((h0 + j) * _DH, _DH)
                    rows = pl.ds(r0, _DH)
                    hr = pl.multiple_of(((h0 + j) % 8) * (_DH // 2), _DH // 2)
                    dsj = ds_sl[slot][j]
                    doe = _upk(wdo_s[0, qb * _H + h0 + j, pl.ds(hr, _DH // 2), :])
                    dom = _upk(wdo_s[1, qb * _H + h0 + j, pl.ds(hr, _DH // 2), :])
                    qtj = _upk(wq_s[qb * _H + h0 + j, pl.ds(hr, _DH // 2), :])
                    dv = jnp.concatenate([_dot(doe, e_s[u, j, 0:QB, :], _NT),
                                          _dot(dom, e_s[u, j, QB:_W, :], _NT),
                                          _dot(doe, e_s[u, j, _W:R, :], _NT)], axis=1)
                    dvt_s[rows, win] += dv
                    dkt_s[rows, win] += _dot(qtj, dsj, _NT)
                    dqt_s[s % 2, rows, pl.ds(qcol, QB)] = _dot(kt_s[rows, win], dsj, _NN) * scale
                return f

            return [mk(j) for j in range(HU)]

        def bhb(u, p, tail):
            q = 1 - p
            a = [] if tail else (ba_steps(u + 2, 2 * q) + ba_steps(u + 3, 2 * q + 1))
            c = bc_steps(u, 2 * p) + bc_steps(u + 1, 2 * p + 1)
            interleave(a, c)

        interleave(ba_steps(0, 0) + ba_steps(1, 1))
        bhb(0, 0, False)

        def bbody(k, carry):
            bhb(4 * k + 2, 1, False)
            bhb(4 * k + 4, 0, False)
            return carry

        lax.fori_loop(0, NU // 4 - 1, bbody, 0)
        bhb(NU - 2, 1, True)

    @pl.when(s > 0)
    def _lag():
        lrow0 = pl.multiple_of((s - 1) * T, T)
        lprow0 = pl.multiple_of((s - 1) * T + _W, 128)
        xl = xl_ref[...].astype(_F32)
        ln1, r1 = _ln_stats(xl)
        ln1b = ln1.astype(_BF16)
        dqkvt = jnp.concatenate([dqt_s[(s - 1) % 2], dkt_s[:, pl.ds(lprow0, T)], dvt_s[:, pl.ds(lprow0, T)]], axis=0)
        dqkv = dqkvt.T.astype(_BF16)
        aqkv[...] += _dot(ln1b, dqkv, _TN)
        dln1 = _dot(dqkv, wqkv_ref[...], _NT)
        dx = dh_s[pl.ds(lrow0, T), :] + _ln_bwd(dln1, ln1, r1)
        dx_ref[...] = dx.astype(dx_ref.dtype)

    @pl.when(s == nblk)
    def _fin():
        dwqkv_ref[...] = aqkv[...].astype(dwqkv_ref.dtype)
        dwo_ref[...] = ao[...].astype(dwo_ref.dtype)
        dwgt_ref[...] = ag[...].T.astype(dwgt_ref.dtype)
        dwut_ref[...] = au[...].T.astype(dwut_ref.dtype)
        dwd_ref[...] = ad[...].astype(dwd_ref.dtype)


@jax.jit
def pallas_sequential_preLN__sliding_block__glu_gated_glu__prompt_kernel(
    A_x: jax.Array,
    A_wqkv: jax.Array,
    A_wo: jax.Array,
    B_x: jax.Array,
    B_w_gate: jax.Array,
    B_w_up: jax.Array,
    B_w_down: jax.Array,
    grad_out: jax.Array,
):
    del B_x
    _, S, D = A_x.shape
    F = B_w_gate.shape[1]
    T, HU = _T, _HU
    nblk = S // T
    NG = D // 128
    NQB = T // _QB
    NU = NQB * (_H // HU)

    cur = lambda s: (0, jnp.minimum(s, nblk - 1), 0)
    lag = lambda s: (0, jnp.maximum(s - 1, 0), 0)
    whole = lambda s: (0, 0)

    in_specs = [
        pl.BlockSpec((None, T, D), cur),
        pl.BlockSpec((None, T, D), lag),
        pl.BlockSpec((None, T, D), cur),
        pl.BlockSpec((D, 3 * D), whole),
        pl.BlockSpec((D, D), whole),
        pl.BlockSpec((F, D), whole),
        pl.BlockSpec((F, D), whole),
        pl.BlockSpec((F, D), whole),
    ]
    out_specs = [
        pl.BlockSpec((None, T, D), cur),
        pl.BlockSpec((None, T, D), lag),
        pl.BlockSpec((D, 3 * D), whole),
        pl.BlockSpec((D, D), whole),
        pl.BlockSpec((F, D), whole),
        pl.BlockSpec((F, D), whole),
        pl.BlockSpec((F, D), whole),
    ]
    out_shape = [
        jax.ShapeDtypeStruct((1, S, D), A_x.dtype),
        jax.ShapeDtypeStruct((1, S, D), A_x.dtype),
        jax.ShapeDtypeStruct((D, 3 * D), A_wqkv.dtype),
        jax.ShapeDtypeStruct((D, D), A_wo.dtype),
        jax.ShapeDtypeStruct((F, D), B_w_gate.dtype),
        jax.ShapeDtypeStruct((F, D), B_w_up.dtype),
        jax.ShapeDtypeStruct((F, D), B_w_down.dtype),
    ]
    scratch_shapes = [
        pltpu.VMEM((NQB * _H, 64, 128), jnp.uint32),
        pltpu.VMEM((2, NQB * _H, 64, 128), jnp.uint32),
        pltpu.VMEM((NG, (S + _W) // 2, 128), jnp.uint32),
        pltpu.VMEM((NG, (S + _W) // 2, 128), jnp.uint32),
        pltpu.VMEM((D, S + _W), _BF16),
        pltpu.VMEM((D, S + _W), _BF16),
        pltpu.VMEM((NU, HU, _R, 128), _BF16),
        pltpu.VMEM((NU, HU, 8, 128), _F32),
        pltpu.VMEM((NU, HU, 8, 128), _F32),
        pltpu.VMEM((NU, HU, 8, 128), _F32),
        pltpu.VMEM((D, T), _F32),
        pltpu.VMEM((HU, _R, 128), _BF16),
        pltpu.VMEM((HU, _R, 128), _BF16),
        pltpu.VMEM((HU, _R, 128), _BF16),
        pltpu.VMEM((HU, _R, 128), _BF16),
        pltpu.VMEM((2, D, T), _F32),
        pltpu.VMEM((D, S + _W), _F32),
        pltpu.VMEM((D, S + _W), _F32),
        pltpu.VMEM((S, D), _F32),
        pltpu.VMEM((D, 3 * D), _F32),
        pltpu.VMEM((D, D), _F32),
        pltpu.VMEM((D, F), _F32),
        pltpu.VMEM((D, F), _F32),
        pltpu.VMEM((F, D), _F32),
    ]
    out, dx, dwqkv, dwo, dwgt, dwut, dwd = pl.pallas_call(
        functools.partial(_kernel, S=S, D=D, T=T, HU=HU),
        grid=(nblk + 1,),
        in_specs=in_specs,
        out_specs=out_specs,
        out_shape=out_shape,
        scratch_shapes=scratch_shapes,
        compiler_params=pltpu.CompilerParams(
            dimension_semantics=("arbitrary",),
            vmem_limit_bytes=110 * 1024 * 1024,
        ),
    )(A_x, A_x, grad_out, A_wqkv, A_wo, B_w_gate.T, B_w_up.T, B_w_down)
    return out, dx, dwqkv, dwo, dwgt.T, dwut.T, dwd
```
